```python
import os as _os
_os.environ.setdefault("JAX_PLATFORMS", "cpu")
import jax
import jax.numpy as jnp

def _softmax(x, axis=-1):
    return jax.nn.softmax(x, axis=axis)
def _gelu(x):
    return jax.nn.gelu(x, approximate=True)
def _silu(x):
    return jax.nn.silu(x)
def _sigmoid(x):
    return jax.nn.sigmoid(x)
def _layernorm(x, axis=-1, eps=1e-5):
    m = jnp.mean(x, axis=axis, keepdims=True)
    v = jnp.var(x, axis=axis, keepdims=True)
    return (x - m) / jnp.sqrt(v + eps)
def _scatter_add(tgt, idx, src, axis=0):
    return tgt.at[idx].add(src)
def _segment_sum(src, seg, n):
    return jax.ops.segment_sum(src, seg, n)
class _Rng:
    def __init__(self, key):
        self._k = key
    def _next(self):
        self._k, sub = jax.random.split(self._k)
        return sub
    def normal(self, shape):
        return jax.random.normal(self._next(), shape, dtype=jnp.bfloat16)
    def randint(self, lo, hi, shape):
        return jax.random.randint(self._next(), shape, lo, hi, dtype=jnp.int32)
    def uniform(self, shape, lo=0.0, hi=1.0):
        return jax.random.uniform(self._next(), shape, jnp.bfloat16, lo, hi)
    def permutation(self, n):
        return jax.random.permutation(self._next(), n)


kernel_name = 'standalone__instancenorm__sampling'

def setup_inputs():
    _rng = _Rng(jax.random.key(int.from_bytes(__import__("os").urandom(4), "little")))
    _w = (lambda a: (lambda t: t.astype(jnp.bfloat16) if jnp.issubdtype(t.dtype, jnp.floating) else t)(jnp.asarray(a)))
    B, C, H, W = 16, 640, 16, 32
    return {
        "x": _w((lambda *s: _rng.normal(s) * 0.05)(B, C, H, W)),
        "g": _w((lambda *s: _rng.normal(s) * 0.05)(C) + 1.0),
        "b": _w((lambda *s: _rng.normal(s) * 0.05)(C)),
    }

def reference(x, g, b):
    mu = x.mean(axis=(-2, -1), keepdims=True)
    var = ((x - mu) * (x - mu)).mean(axis=(-2, -1), keepdims=True)
    xhat = (x - mu) / jnp.sqrt(var + 1e-5)
    return xhat * g.reshape(1, -1, 1, 1) + b.reshape(1, -1, 1, 1)
```

```python
import jax
import jax.numpy as jnp
import jax.experimental.pallas as pl
import jax.experimental.pallas.tpu as pltpu

_EPS = 1e-5


@jax.jit
def pallas_standalone__instancenorm__sampling_kernel(
    x: jax.Array,
    g: jax.Array,
    b: jax.Array,
):
    B, C, H, W = x.shape
    HW = H * W

    def kernel_function(x_ref, g_ref, b_ref, o_ref):
        xf = x_ref[...].astype(jnp.float32)
        gf = g_ref[...].astype(jnp.float32).reshape(1, C)
        bf = b_ref[...].astype(jnp.float32).reshape(1, C)
        mu = jnp.sum(xf, axis=0, keepdims=True) * (1.0 / HW)
        d = xf - mu
        var = jnp.sum(d * d, axis=0, keepdims=True) * (1.0 / HW)
        a = gf * jax.lax.rsqrt(var + _EPS)
        o_ref[...] = (d * a + bf).astype(o_ref.dtype)

    xt = x.transpose(0, 2, 3, 1).reshape(B, HW, C)
    out = pl.pallas_call(
        kernel_function,
        grid=(B,),
        in_specs=[
            pl.BlockSpec((None, HW, C), lambda i: (i, 0, 0)),
            pl.BlockSpec((C,), lambda i: (0,)),
            pl.BlockSpec((C,), lambda i: (0,)),
        ],
        out_specs=pl.BlockSpec((None, HW, C), lambda i: (i, 0, 0)),
        out_shape=jax.ShapeDtypeStruct((B, HW, C), x.dtype),
        compiler_params=pltpu.CompilerParams(dimension_semantics=("parallel",)),
    )(xt, g, b)
    return out.reshape(B, H, W, C).transpose(0, 3, 1, 2)
```

```python
import jax
import jax.numpy as jnp
import jax.experimental.pallas as pl
import jax.experimental.pallas.tpu as pltpu

_EPS = 1e-5
_LANES = 128
_READ_AHEAD = 5
_READ_CHUNK = 8
_WRITE_CHUNK = 16
_WRITE_GROUP = 4
_WRITE_START = 13


@jax.jit
def pallas_standalone__instancenorm__sampling_kernel(
    x: jax.Array,
    g: jax.Array,
    b: jax.Array,
):
    B, C, H, W = x.shape
    HW = H * W
    NJ = C // _LANES
    U = HW * C // (16 * _LANES)
    NP = U // NJ
    K = _READ_AHEAD
    HALF = U // 2

    def normalise(xbuf, obuf, u0, gs, bs):
        v = xbuf[pl.ds(u0, U)].astype(jnp.float32).reshape(NP, NJ, 16, _LANES)

        def tile(t):
            lo = (t % 2) * 8
            return v[:, t // 2, lo:lo + 8, :]

        outs = {}
        for j in range(NJ):
            t1, t2 = tile(j), tile(j + NJ)
            s = jnp.sum(t1, axis=0) + jnp.sum(t2, axis=0)
            mu = jnp.sum(s, axis=0, keepdims=True) * (1.0 / HW)
            d1, d2 = t1 - mu, t2 - mu
            q = jnp.sum(d1 * d1, axis=0) + jnp.sum(d2 * d2, axis=0)
            var = jnp.sum(q, axis=0, keepdims=True) * (1.0 / HW)
            a = gs[j] * jax.lax.rsqrt(var + _EPS)
            outs[j] = d1 * a + bs[j]
            outs[j + NJ] = d2 * a + bs[j]
        o = jnp.stack(
            [jnp.concatenate([outs[2 * p], outs[2 * p + 1]], axis=1) for p in range(NJ)],
            axis=1,
        )
        obuf[pl.ds(u0, U)] = o.reshape(U, 16, _LANES).astype(obuf.dtype)

    def kernel_function(x_hbm, g_hbm, b_hbm, o_hbm, xbuf, obuf, gbuf, bbuf, sem):
        osem = sem.at[K]

        def read_start(i):
            def chunk(c, carry):
                for s in range(2):
                    o = i * U + s * HALF + c * _READ_CHUNK
                    pltpu.make_async_copy(
                        x_hbm.at[pl.ds(o, _READ_CHUNK)],
                        xbuf.at[pl.ds(o, _READ_CHUNK)],
                        sem.at[i % K],
                    ).start(priority=s)
                return carry

            jax.lax.fori_loop(0, HALF // _READ_CHUNK, chunk, 0)

        def read_wait(i):
            pltpu.make_async_copy(
                x_hbm.at[pl.ds(i * U, U)], xbuf.at[pl.ds(i * U, U)], sem.at[i % K]
            ).wait()

        def write_group(gi, carry):
            def chunk(c, carry2):
                for s in range(_WRITE_GROUP):
                    o = (gi * _WRITE_GROUP + s) * U + c * _WRITE_CHUNK
                    pltpu.make_async_copy(
                        obuf.at[pl.ds(o, _WRITE_CHUNK)],
                        o_hbm.at[pl.ds(o, _WRITE_CHUNK)],
                        osem,
                    ).start(priority=s % 2)
                return carry2

            jax.lax.fori_loop(0, U // _WRITE_CHUNK, chunk, 0)
            return carry

        read_start(0)
        g_copy = pltpu.make_async_copy(g_hbm, gbuf, osem)
        b_copy = pltpu.make_async_copy(b_hbm, bbuf, osem)
        g_copy.start()
        b_copy.start()

        def first_reads(i, carry):
            read_start(i)
            return carry

        jax.lax.fori_loop(1, K, first_reads, 0)
        g_copy.wait()
        b_copy.wait()
        gf = gbuf[...].astype(jnp.float32).reshape(1, C)
        bf = bbuf[...].astype(jnp.float32).reshape(1, C)
        gs = [gf[:, j * _LANES:(j + 1) * _LANES] for j in range(NJ)]
        bs = [bf[:, j * _LANES:(j + 1) * _LANES] for j in range(NJ)]

        early_groups = _WRITE_START // _WRITE_GROUP

        def per_batch(i, carry):
            read_wait(i)

            @pl.when(i + K < B)
            def _():
                read_start(i + K)

            @pl.when(i == _WRITE_START)
            def _():
                jax.lax.fori_loop(0, early_groups, write_group, 0)

            normalise(xbuf, obuf, i * U, gs, bs)
            return carry

        jax.lax.fori_loop(0, B, per_batch, 0)
        jax.lax.fori_loop(early_groups, B // _WRITE_GROUP, write_group, 0)
        pltpu.make_async_copy(obuf, o_hbm, osem).wait()

    xv = (
        x.reshape(B, NJ, _LANES, H, W // 8, 8)
        .transpose(0, 3, 4, 1, 5, 2)
        .reshape(B * U, 16, _LANES)
    )
    out = pl.pallas_call(
        kernel_function,
        in_specs=[pl.BlockSpec(memory_space=pl.ANY)] * 3,
        out_specs=pl.BlockSpec(memory_space=pl.ANY),
        out_shape=jax.ShapeDtypeStruct((B * U, 16, _LANES), x.dtype),
        scratch_shapes=[
            pltpu.VMEM((B * U, 16, _LANES), x.dtype),
            pltpu.VMEM((B * U, 16, _LANES), x.dtype),
            pltpu.VMEM((C,), g.dtype),
            pltpu.VMEM((C,), b.dtype),
            pltpu.SemaphoreType.DMA((K + 1,)),
        ],
        compiler_params=pltpu.CompilerParams(vmem_limit_bytes=64 * 1024 * 1024),
    )(xv, g, b)
    return (
        out.reshape(B, H, W // 8, NJ, 8, _LANES)
        .transpose(0, 3, 5, 1, 2, 4)
        .reshape(B, C, H, W)
    )
```

```python
import jax
import jax.numpy as jnp
import jax.experimental.pallas as pl
import jax.experimental.pallas.tpu as pltpu

_EPS = 1e-5
_LANES = 128
_READ_AHEAD = 5
_READ_CHUNK = 8
_WRITE_CHUNK = 16
_WRITE_GROUP = 4
_WRITE_START = 13
_WRITE_PHASE = 12


@jax.jit
def pallas_standalone__instancenorm__sampling_kernel(
    x: jax.Array,
    g: jax.Array,
    b: jax.Array,
):
    B, C, H, W = x.shape
    HW = H * W
    NJ = C // _LANES
    U = HW * C // (16 * _LANES)
    NP = U // NJ
    K = _READ_AHEAD
    HALF = U // 2

    def normalise(xbuf, obuf, u0, gs, bs):
        v = xbuf[pl.ds(u0, U)].astype(jnp.float32).reshape(NP, NJ, 16, _LANES)

        def tile(t):
            lo = (t % 2) * 8
            return v[:, t // 2, lo:lo + 8, :]

        outs = {}
        for j in range(NJ):
            t1, t2 = tile(j), tile(j + NJ)
            s = jnp.sum(t1, axis=0) + jnp.sum(t2, axis=0)
            mu = jnp.sum(s, axis=0, keepdims=True) * (1.0 / HW)
            d1, d2 = t1 - mu, t2 - mu
            q = jnp.sum(d1 * d1, axis=0) + jnp.sum(d2 * d2, axis=0)
            var = jnp.sum(q, axis=0, keepdims=True) * (1.0 / HW)
            a = gs[j] * jax.lax.rsqrt(var + _EPS)
            outs[j] = d1 * a + bs[j]
            outs[j + NJ] = d2 * a + bs[j]
        o = jnp.stack(
            [jnp.concatenate([outs[2 * p], outs[2 * p + 1]], axis=1) for p in range(NJ)],
            axis=1,
        )
        obuf[pl.ds(u0, U)] = o.reshape(U, 16, _LANES).astype(obuf.dtype)

    def kernel_function(x_hbm, g_hbm, b_hbm, o_hbm, xbuf, obuf, gbuf, bbuf, sem):
        osem = sem.at[K]

        def read_start(i):
            def chunk(c, carry):
                for s in range(2):
                    o = i * U + s * HALF + c * _READ_CHUNK
                    pltpu.make_async_copy(
                        x_hbm.at[pl.ds(o, _READ_CHUNK)],
                        xbuf.at[pl.ds(o, _READ_CHUNK)],
                        sem.at[i % K],
                    ).start(priority=s)
                return carry

            jax.lax.fori_loop(0, HALF // _READ_CHUNK, chunk, 0)

        def read_wait(i):
            pltpu.make_async_copy(
                x_hbm.at[pl.ds(i * U, U)], xbuf.at[pl.ds(i * U, U)], sem.at[i % K]
            ).wait()

        def write_copy(o, n):
            return pltpu.make_async_copy(
                obuf.at[pl.ds(o, n)], o_hbm.at[pl.ds(o, n)], osem
            )

        n_groups = B // _WRITE_GROUP
        n_chunks = U // _WRITE_CHUNK
        tail = _WRITE_CHUNK - _WRITE_PHASE

        def write_group(gi, carry):
            def chunk(c, carry2):
                for s in range(_WRITE_GROUP):
                    o = _WRITE_PHASE + (gi * _WRITE_GROUP + s) * U + c * _WRITE_CHUNK
                    if s < _WRITE_GROUP - 1:
                        write_copy(o, _WRITE_CHUNK).start(priority=s % 2)
                    else:
                        @pl.when(jnp.logical_or(gi < n_groups - 1, c < n_chunks - 1))
                        def _():
                            write_copy(o, _WRITE_CHUNK).start(priority=s % 2)
                return carry2

            jax.lax.fori_loop(0, n_chunks, chunk, 0)
            return carry

        read_start(0)
        g_copy = pltpu.make_async_copy(g_hbm, gbuf, osem)
        b_copy = pltpu.make_async_copy(b_hbm, bbuf, osem)
        g_copy.start()
        b_copy.start()

        def first_reads(i, carry):
            read_start(i)
            return carry

        jax.lax.fori_loop(1, K, first_reads, 0)
        g_copy.wait()
        b_copy.wait()
        gf = gbuf[...].astype(jnp.float32).reshape(1, C)
        bf = bbuf[...].astype(jnp.float32).reshape(1, C)
        gs = [gf[:, j * _LANES:(j + 1) * _LANES] for j in range(NJ)]
        bs = [bf[:, j * _LANES:(j + 1) * _LANES] for j in range(NJ)]

        early_groups = _WRITE_START // _WRITE_GROUP

        def per_batch(i, carry):
            read_wait(i)

            @pl.when(i + K < B)
            def _():
                read_start(i + K)

            @pl.when(i == _WRITE_START)
            def _():
                jax.lax.fori_loop(0, early_groups, write_group, 0)

            normalise(xbuf, obuf, i * U, gs, bs)
            return carry

        jax.lax.fori_loop(0, B, per_batch, 0)
        jax.lax.fori_loop(early_groups, n_groups, write_group, 0)
        write_copy(B * U - tail, tail).start(priority=0)
        write_copy(0, _WRITE_PHASE).start(priority=1)
        pltpu.make_async_copy(obuf, o_hbm, osem).wait()

    xv = (
        x.reshape(B, NJ, _LANES, H, W // 8, 8)
        .transpose(0, 3, 4, 1, 5, 2)
        .reshape(B * U, 16, _LANES)
    )
    out = pl.pallas_call(
        kernel_function,
        in_specs=[pl.BlockSpec(memory_space=pl.ANY)] * 3,
        out_specs=pl.BlockSpec(memory_space=pl.ANY),
        out_shape=jax.ShapeDtypeStruct((B * U, 16, _LANES), x.dtype),
        scratch_shapes=[
            pltpu.VMEM((B * U, 16, _LANES), x.dtype),
            pltpu.VMEM((B * U, 16, _LANES), x.dtype),
            pltpu.VMEM((C,), g.dtype),
            pltpu.VMEM((C,), b.dtype),
            pltpu.SemaphoreType.DMA((K + 1,)),
        ],
        compiler_params=pltpu.CompilerParams(vmem_limit_bytes=64 * 1024 * 1024),
    )(xv, g, b)
    return (
        out.reshape(B, H, W // 8, NJ, 8, _LANES)
        .transpose(0, 3, 5, 1, 2, 4)
        .reshape(B, C, H, W)
    )
```

```python
import jax
import jax.numpy as jnp
import jax.experimental.pallas as pl
import jax.experimental.pallas.tpu as pltpu

_EPS = 1e-5
_LANES = 128
_UNIT_ROWS = 16

_READ_GROUP = 2
_READ_AHEAD = 3
_READ_CHUNK = 8
_WRITE_GROUP = 8
_WRITE_CHUNK = 4
_WRITE_START = 12
_WRITE_FIRST = 10
_WRITE_EACH = 4


@jax.jit
def pallas_standalone__instancenorm__sampling_kernel(
    x: jax.Array,
    g: jax.Array,
    b: jax.Array,
):
    B, C, H, W = x.shape
    HW = H * W
    NJ = C // _LANES
    U = HW * C // (_UNIT_ROWS * _LANES)
    NP = U // NJ
    HALF = U // 2
    n_read_groups = B // _READ_GROUP
    n_write_groups = B // _WRITE_GROUP
    n_write_steps = U // _WRITE_CHUNK

    def normalise(xbuf, obuf, u0, gs, bs):
        v = xbuf[pl.ds(u0, U)].astype(jnp.float32).reshape(NP, NJ, _UNIT_ROWS, _LANES)

        def tile(t):
            lo = (t % 2) * 8
            return v[:, t // 2, lo:lo + 8, :]

        outs = {}
        for j in range(NJ):
            t1, t2 = tile(j), tile(j + NJ)
            s = jnp.sum(t1, axis=0) + jnp.sum(t2, axis=0)
            mu = jnp.sum(s, axis=0, keepdims=True) * (1.0 / HW)
            d1, d2 = t1 - mu, t2 - mu
            q = jnp.sum(d1 * d1, axis=0) + jnp.sum(d2 * d2, axis=0)
            var = jnp.sum(q, axis=0, keepdims=True) * (1.0 / HW)
            a = gs[j] * jax.lax.rsqrt(var + _EPS)
            outs[j] = d1 * a + bs[j]
            outs[j + NJ] = d2 * a + bs[j]
        o = jnp.stack(
            [jnp.concatenate([outs[2 * p], outs[2 * p + 1]], axis=1) for p in range(NJ)],
            axis=1,
        )
        obuf[pl.ds(u0, U)] = o.reshape(U, _UNIT_ROWS, _LANES).astype(obuf.dtype)

    def kernel_function(x_hbm, g_hbm, b_hbm, o_hbm, xbuf, obuf, gbuf, bbuf, sem):
        osem = sem.at[_READ_AHEAD]

        def read_start(gi):
            def step(c, carry):
                for s in range(2 * _READ_GROUP):
                    o = gi * (_READ_GROUP * U) + s * HALF + c * _READ_CHUNK
                    pltpu.make_async_copy(
                        x_hbm.at[pl.ds(o, _READ_CHUNK)],
                        xbuf.at[pl.ds(o, _READ_CHUNK)],
                        sem.at[gi % _READ_AHEAD],
                    ).start(priority=s % 2)
                return carry

            jax.lax.fori_loop(0, HALF // _READ_CHUNK, step, 0)

        def read_wait(gi):
            span = pl.ds(gi * (_READ_GROUP * U), _READ_GROUP * U)
            pltpu.make_async_copy(
                x_hbm.at[span], xbuf.at[span], sem.at[gi % _READ_AHEAD]
            ).wait()

        def write_steps(gi, lo, hi):
            def step(c, carry):
                for s in range(_WRITE_GROUP):
                    o = (gi * _WRITE_GROUP + s) * U + c * _WRITE_CHUNK
                    pltpu.make_async_copy(
                        obuf.at[pl.ds(o, _WRITE_CHUNK)],
                        o_hbm.at[pl.ds(o, _WRITE_CHUNK)],
                        osem,
                    ).start(priority=s % 2)
                return carry

            jax.lax.fori_loop(lo, hi, step, 0)

        read_start(0)
        g_copy = pltpu.make_async_copy(g_hbm, gbuf, osem)
        b_copy = pltpu.make_async_copy(b_hbm, bbuf, osem)
        g_copy.start()
        b_copy.start()

        def first_reads(gi, carry):
            read_start(gi)
            return carry

        jax.lax.fori_loop(1, _READ_AHEAD, first_reads, 0)
        g_copy.wait()
        b_copy.wait()
        gf = gbuf[...].astype(jnp.float32).reshape(1, C)
        bf = bbuf[...].astype(jnp.float32).reshape(1, C)
        gs = [gf[:, j * _LANES:(j + 1) * _LANES] for j in range(NJ)]
        bs = [bf[:, j * _LANES:(j + 1) * _LANES] for j in range(NJ)]

        def per_batch(i, carry):
            @pl.when(i % _READ_GROUP == 0)
            def _():
                gi = i // _READ_GROUP
                read_wait(gi)

                @pl.when(gi + _READ_AHEAD < n_read_groups)
                def _():
                    read_start(gi + _READ_AHEAD)

            @pl.when(i == _WRITE_START)
            def _():
                write_steps(0, 0, _WRITE_FIRST)

            normalise(xbuf, obuf, i * U, gs, bs)

            @pl.when(jnp.logical_and(i >= _WRITE_START, i < B - 1))
            def _():
                lo = _WRITE_FIRST + (i - _WRITE_START) * _WRITE_EACH
                write_steps(0, lo, lo + _WRITE_EACH)

            return carry

        jax.lax.fori_loop(0, B, per_batch, 0)

        write_steps(0, _WRITE_FIRST + (B - 1 - _WRITE_START) * _WRITE_EACH, n_write_steps)

        def later_groups(gi, carry):
            write_steps(gi, 0, n_write_steps)
            return carry

        jax.lax.fori_loop(1, n_write_groups, later_groups, 0)
        pltpu.make_async_copy(obuf, o_hbm, osem).wait()

    xv = (
        x.reshape(B, NJ, _LANES, H, W // 8, 8)
        .transpose(0, 3, 4, 1, 5, 2)
        .reshape(B * U, _UNIT_ROWS, _LANES)
    )
    out = pl.pallas_call(
        kernel_function,
        in_specs=[pl.BlockSpec(memory_space=pl.ANY)] * 3,
        out_specs=pl.BlockSpec(memory_space=pl.ANY),
        out_shape=jax.ShapeDtypeStruct((B * U, _UNIT_ROWS, _LANES), x.dtype),
        scratch_shapes=[
            pltpu.VMEM((B * U, _UNIT_ROWS, _LANES), x.dtype),
            pltpu.VMEM((B * U, _UNIT_ROWS, _LANES), x.dtype),
            pltpu.VMEM((C,), g.dtype),
            pltpu.VMEM((C,), b.dtype),
            pltpu.SemaphoreType.DMA((_READ_AHEAD + 1,)),
        ],
        compiler_params=pltpu.CompilerParams(vmem_limit_bytes=64 * 1024 * 1024),
    )(xv, g, b)
    return (
        out.reshape(B, H, W // 8, NJ, 8, _LANES)
        .transpose(0, 3, 5, 1, 2, 4)
        .reshape(B, C, H, W)
    )
```
